```python
import jax
import jax.numpy as jnp

def _softmax(x, axis=-1):
    return jax.nn.softmax(x, axis=axis)

def _gelu(x):
    return jax.nn.gelu(x, approximate=True)

def _silu(x):
    return jax.nn.silu(x)

def _sigmoid(x):
    return jax.nn.sigmoid(x)

def _layernorm(x, axis=-1, eps=1e-05):
    m = jnp.mean(x, axis=axis, keepdims=True)
    v = jnp.var(x, axis=axis, keepdims=True)
    return (x - m) / jnp.sqrt(v + eps)

def _scatter_add(tgt, idx, src, axis=0):
    return tgt.at[idx].add(src)

def _segment_sum(src, seg, n):
    return jax.ops.segment_sum(src, seg, n)

class _Rng:

    def __init__(self, key):
        self._k = key

    def _next(self):
        self._k, sub = jax.random.split(self._k)
        return sub

    def normal(self, shape):
        return jax.random.normal(self._next(), shape, dtype=jnp.bfloat16)

    def randint(self, lo, hi, shape):
        return jax.random.randint(self._next(), shape, lo, hi, dtype=jnp.int32)

    def uniform(self, shape, lo=0.0, hi=1.0):
        return jax.random.uniform(self._next(), shape, jnp.bfloat16, lo, hi)

    def permutation(self, n):
        return jax.random.permutation(self._next(), n)
kernel_name = 'sequential_preLN__memory_aug_recurrent_mem_tr__mixer_s_mlp__prompt'

def setup_inputs():
    _rng = _Rng(jax.random.key(int.from_bytes(__import__("os").urandom(4), "little")))
    _w = lambda a: (lambda t: t.astype(jnp.bfloat16) if jnp.issubdtype(t.dtype, jnp.floating) else t)(jnp.asarray(a))

    def _A_setup():
        B, S, Dm = (1, 2048, 1024)
        H, Dh = (32, 128)
        M, seg = (8, 32)
        seg = min(seg, S)
        S = S // seg * seg
        return {'x': _w((lambda *s: _rng.normal(s) * 0.05)(B, S, Dm)), 'mem0': _w((lambda *s: _rng.normal(s) * 0.05)(B, M, Dm)), 'Wq': _w((lambda *s: _rng.normal(s) * 0.05)(Dm, H, Dh) * Dm ** (-0.5)), 'Wk': _w((lambda *s: _rng.normal(s) * 0.05)(Dm, H, Dh) * Dm ** (-0.5)), 'Wv': _w((lambda *s: _rng.normal(s) * 0.05)(Dm, H, Dh) * Dm ** (-0.5)), 'Wo': _w((lambda *s: _rng.normal(s) * 0.05)(H, Dh, Dm) * (H * Dh) ** (-0.5)), 'seg_len': seg}
    _A_in = _A_setup()

    def _B_setup():
        B, S, D, F = (1, 2048, 1024, 3584)
        return {'x': _w((lambda *s: _rng.normal(s) * 0.05)(B, S, D)), 'w1': _w((lambda *s: _rng.normal(s) * 0.05)(D, D) * D ** (-0.5)), 'w2': _w((lambda *s: _rng.normal(s) * 0.05)(D, D) * D ** (-0.5)), 'w3': _w((lambda *s: _rng.normal(s) * 0.05)(D, F) * D ** (-0.5)), 'w4': _w((lambda *s: _rng.normal(s) * 0.05)(F, D) * F ** (-0.5))}
    _B_in = _B_setup()
    return {'A_x': _A_in['x'], 'A_mem0': _A_in['mem0'], 'A_Wq': _A_in['Wq'], 'A_Wk': _A_in['Wk'], 'A_Wv': _A_in['Wv'], 'A_Wo': _A_in['Wo'], 'A_seg_len': _A_in['seg_len'], 'B_x': _B_in['x'], 'B_w1': _B_in['w1'], 'B_w2': _B_in['w2'], 'B_w3': _B_in['w3'], 'B_w4': _B_in['w4']}

def reference(A_x, A_mem0, A_Wq, A_Wk, A_Wv, A_Wo, A_seg_len, B_x, B_w1, B_w2, B_w3, B_w4):

    def _A_ref(x, mem0, Wq, Wk, Wv, Wo, seg_len):
        B, S, Dm = x.shape
        H, Dh = (Wq.shape[1], Wq.shape[2])
        M = mem0.shape[1]
        scale = Dh ** (-0.5)
        n_seg = S // seg_len
        L = M + seg_len
        idx = jnp.arange(L)
        mask = (idx[:, None] < M) | (idx[:, None] >= idx[None, :])
        mem = mem0
        outs = []
        for s in range(n_seg):
            xs = x[:, s * seg_len:(s + 1) * seg_len, :].copy()
            h = jnp.concatenate([mem, xs], axis=1)
            q = jnp.einsum('btd,dhe->bhte', h, Wq)
            k = jnp.einsum('btd,dhe->bhte', h, Wk)
            v = jnp.einsum('btd,dhe->bhte', h, Wv)
            scores = jnp.einsum('bhqe,bhke->bhqk', q, k) * scale
            scores = jnp.where(mask[None, None], scores, -1000000000.0)
            p = _softmax(scores, axis=-1)
            o = jnp.einsum('bhqk,bhke->bhqe', p, v)
            o = jnp.einsum('bhte,hed->btd', o, Wo)
            mem = o[:, :M, :].copy()
            outs.append(o[:, M:, :])
        return jnp.concatenate(outs, axis=1)

    def _B_ref(x, w1, w2, w3, w4):
        B, S, D = x.shape
        h = _gelu(_layernorm(x, axis=-1) @ w1)
        c = D // 4
        g0 = jnp.pad(h[:, :, 0 * c:1 * c], ((0, 0), (1, 0), (0, 0)))[:, :S, :]
        g1 = jnp.pad(h[:, :, 1 * c:2 * c], ((0, 0), (0, 1), (0, 0)))[:, 1:, :]
        g2 = jnp.pad(h[:, :, 2 * c:3 * c], ((0, 0), (2, 0), (0, 0)))[:, :S, :]
        g3 = jnp.pad(h[:, :, 3 * c:], ((0, 0), (0, 2), (0, 0)))[:, 2:, :]
        hs = jnp.concatenate([g0, g1, g2, g3], axis=-1) @ w2
        x1 = x + hs
        h2 = _gelu(_layernorm(x1, axis=-1) @ w3) @ w4
        return x1 + h2
    x = A_x
    h = x + _A_ref(_layernorm(x, axis=-1), A_mem0, A_Wq, A_Wk, A_Wv, A_Wo, A_seg_len)
    h2 = h + _B_ref(_layernorm(h, axis=-1), B_w1, B_w2, B_w3, B_w4)
    return h2
```

```python
import functools
import math

import jax
import jax.numpy as jnp
from jax import lax
from jax.experimental import pallas as pl
from jax.experimental.pallas import tpu as pltpu

F32 = jnp.float32
BF16 = jnp.bfloat16
I32 = jnp.int32

LN_EPS = 1e-5
NEG = -1000000000.0


def _layernorm(x):
    m = jnp.mean(x, axis=-1, keepdims=True)
    c = x - m
    v = jnp.mean(c * c, axis=-1, keepdims=True)
    return c * lax.rsqrt(v + LN_EPS)


def _gelu(x):
    c0 = math.sqrt(2.0 / math.pi)
    u = x * (c0 + (c0 * 0.044715) * (x * x))
    return (0.5 * x) * (1.0 + jnp.tanh(u))


SCHED = 'pipe'
GH = 4


def _make_kernel(S, D, H, E, M, SEG, FF):
    NSEG = S // SEG
    LEFT = 8
    MAIN = SEG - LEFT
    NL = NSEG * LEFT
    L = M + SEG
    HE = H * E
    KC = 128
    NKC = D // KC
    NSTAGE = 2
    RB = 256
    scale = float(E) ** -0.5

    def kernel(x_hbm, mem_hbm, wq_hbm, wk_hbm, wv_hbm, wo_hbm, w1_hbm, w2_hbm, w3_hbm, w4_hbm,
               out_hbm,
               xs, mems, hbuf, w1, w2, w3, w4, sem_in, sem_b, sem_out):

        def phase_a(stage, wqkv, wo, lqkv, lo, qkv_s, s_s, p_s, o_s, sem_st, sem_wo):
            x_cp = pltpu.make_async_copy(x_hbm, xs, sem_in.at[0])
            m_cp = pltpu.make_async_copy(mem_hbm, mems, sem_in.at[1])
            x_cp.start()
            m_cp.start()
            w_hbms = (wq_hbm, wk_hbm, wv_hbm)

            def st_copy(i):
                m, c = divmod(i, NKC)
                return pltpu.make_async_copy(
                    w_hbms[m].at[pl.ds(c * KC * H, KC * H), :], stage.at[i % NSTAGE], sem_st.at[i % NSTAGE])

            def relayout(i):
                m, c = divmod(i, NKC)
                st = stage.at[i % NSTAGE].bitcast(I32)

                def body(g, carry):
                    base = pl.multiple_of(g * (16 * H // 2), 16 * H // 2)
                    sub = st.at[pl.ds(base, 16 * H // 2), :]
                    orow = pl.multiple_of(c * (KC // 2) + g * 8, 8)
                    for hp in range(H // 2):
                        ev = sub[pl.ds(hp, 8, stride=H), :]
                        od = sub[pl.ds(hp + H // 2, 8, stride=H), :]
                        wqkv[m * H + 2 * hp, pl.ds(orow, 8), :] = (ev & 0xFFFF) | (od << 16)
                        wqkv[m * H + 2 * hp + 1, pl.ds(orow, 8), :] = (
                            lax.shift_right_logical(ev, 16) | (od & jnp.int32(-65536)))
                    return carry
                lax.fori_loop(0, KC // 16, body, 0)

            for i in range(NSTAGE):
                st_copy(i).start()
            wo_cps = [pltpu.make_async_copy(wo_hbm.at[:, pl.ds(j * 128, 128)], wo.at[j], sem_wo.at[j])
                      for j in range(D // 128)]
            b_cps = [pltpu.make_async_copy(a, b, sem_b.at[j])
                     for j, (a, b) in enumerate(((w1_hbm, w1), (w2_hbm, w2), (w3_hbm, w3), (w4_hbm, w4)))]
            nst = 3 * NKC
            with jax.named_scope("PH_load"):
                for i in range(nst):
                    st_copy(i).wait()
                    relayout(i)
                    if i + NSTAGE < nst:
                        st_copy(i + NSTAGE).start()
                    elif i + NSTAGE == nst:
                        for cp in wo_cps:
                            cp.start()
                        for cp in b_cps:
                            cp.start()
                x_cp.wait()
                m_cp.wait()

            def w_head(j):
                return pltpu.bitcast(wqkv[j], BF16)

            xl = jnp.concatenate(
                [xs[s * SEG + MAIN:(s + 1) * SEG, :].astype(F32) for s in range(NSEG)], axis=0)
            xl = _layernorm(xl).astype(BF16)
            with jax.named_scope("PH_left"):
                for m in range(3):
                    for hg in range(H // 4):
                        w = jnp.concatenate([w_head(m * H + hg * 4 + t) for t in range(4)], axis=1)
                        lqkv[m, :, hg * 4 * E:(hg + 1) * 4 * E] = jnp.dot(xl, w, preferred_element_type=F32)

            for cp in wo_cps:
                cp.wait()

            def wo_full():
                return jnp.concatenate([wo[j] for j in range(D // 128)], axis=1)

            LP = 128
            row = lax.broadcasted_iota(I32, (L, LP), 0)
            col = lax.broadcasted_iota(I32, (L, LP), 1)
            valid = (col < L) & ((row < M) | (row >= col))
            fill = jnp.where(col < L, NEG / scale, -jnp.inf).astype(F32)
            c_exp = scale * math.log2(math.e)
            RM = M + MAIN

            def step(s, mem):
                r0 = pl.multiple_of(s * SEG, SEG)
                l0 = pl.multiple_of(s * LEFT, LEFT)
                xr = xs[pl.ds(r0, MAIN), :].astype(F32)
                lhs = jnp.concatenate([mem, _layernorm(xr)], axis=0).astype(BF16)

                def proj(h):
                    w = jnp.concatenate([w_head(h), w_head(H + h), w_head(2 * H + h)], axis=1)
                    qkv = jnp.dot(lhs, w, preferred_element_type=F32).astype(BF16)
                    for m in range(3):
                        qkv_s[m * H + h] = pltpu.bitcast(qkv[:, m * E:(m + 1) * E], I32)

                def full(m, h, rows):
                    main = pltpu.bitcast(qkv_s[m * H + h], BF16)
                    left = jnp.concatenate(
                        [lqkv[m, pl.ds(l0, LEFT), h * E:(h + 1) * E], jnp.zeros((8, E), F32)], axis=0).astype(BF16)
                    parts = [main, left]
                    if rows > RM + 16:
                        parts.append(jnp.zeros((rows - RM - 16, E), BF16))
                    return jnp.concatenate(parts, axis=0)

                def scores(h):
                    q = full(0, h, RM + 16)
                    k = full(1, h, LP)
                    sc = lax.dot_general(q, k, (((1,), (1,)), ((), ())), preferred_element_type=F32)
                    s_s[h] = sc[:L]

                def softmax(h):
                    sc = jnp.where(valid, s_s[h], fill)
                    mx = jnp.max(sc, axis=-1, keepdims=True)
                    e = jnp.exp2((sc - mx) * c_exp)
                    sm = jnp.sum(e, axis=-1, keepdims=True)
                    p = e * pl.reciprocal(sm, approx=True)
                    p = jnp.concatenate([p, jnp.zeros((8, LP), F32)], axis=0).astype(BF16)
                    p_s[h] = pltpu.bitcast(p, I32)

                def pv(h):
                    p = pltpu.bitcast(p_s[h], BF16)
                    v = full(2, h, LP)
                    o = jnp.dot(p, v, preferred_element_type=F32)
                    lo[pl.ds(l0, LEFT), h * E:(h + 1) * E] = o[RM:L, :]
                    o_s[:, h * E:(h + 1) * E] = pltpu.bitcast(o[:RM].astype(BF16), I32)

                NG = H // GH
                def grp(f, g):
                    if 0 <= g < NG:
                        for h in range(g * GH, (g + 1) * GH):
                            f(h)
                if SCHED == "stage":
                    for f in (proj, scores, softmax, pv):
                        for h in range(H):
                            f(h)
                else:
                    for t in range(NG + 3):
                        grp(proj, t)
                        grp(scores, t - 1)
                        grp(softmax, t - 2)
                        grp(pv, t - 3)

                o_all = pltpu.bitcast(o_s[...], BF16)
                out = jnp.dot(o_all, wo_full(), preferred_element_type=F32)
                hbuf[pl.ds(r0, MAIN), :] = xr + out[M:, :]
                return out[:M, :]

            with jax.named_scope("PH_main"):
                lax.fori_loop(0, NSEG, step, mems[...].astype(F32))

            with jax.named_scope("PH_oleft"):
                ol = jnp.dot(lo[...].astype(BF16), wo_full(), preferred_element_type=F32)
                for s in range(NSEG):
                    r = s * SEG + MAIN
                    hbuf[r:r + LEFT, :] = xs[r:r + LEFT, :].astype(F32) + ol[s * LEFT:(s + 1) * LEFT, :]
            for cp in b_cps:
                cp.wait()

        pl.run_scoped(
            phase_a,
            pltpu.VMEM((NSTAGE, KC * H, E), BF16),
            pltpu.VMEM((3 * H, D // 2, E), I32),
            pltpu.VMEM((D // 128, HE, 128), BF16),
            pltpu.VMEM((3, NL, HE), F32),
            pltpu.VMEM((NL, HE), F32),
            pltpu.VMEM((3 * H, (M + MAIN) // 2, E), I32),
            pltpu.VMEM((H, L, 128), F32),
            pltpu.VMEM((H, 24, 128), I32),
            pltpu.VMEM(((M + MAIN) // 2, HE), I32),
            pltpu.SemaphoreType.DMA((NSTAGE,)),
            pltpu.SemaphoreType.DMA((D // 128,)),
        )

        def phase_b(g, obuf):
            C = D // 4
            zeros = jnp.zeros((8, D), F32)
            g[0:8, :] = zeros
            g[S + 8:S + 16, :] = zeros

            def b1(j, carry):
                r0 = pl.multiple_of(j * RB, RB)
                hn = _layernorm(hbuf[pl.ds(r0, RB), :])
                a = jnp.dot(hn.astype(BF16), w1[...], preferred_element_type=F32)
                g[pl.ds(r0 + 8, RB), :] = _gelu(a)
                return carry
            with jax.named_scope("PH_b1"):
                lax.fori_loop(0, S // RB, b1, 0)

            def out_copy(j, slot):
                return pltpu.make_async_copy(obuf.at[slot], out_hbm.at[pl.ds(j * RB, RB), :], sem_out.at[slot])

            def b2(j, carry):
                r0 = pl.multiple_of(j * RB, RB)
                slot = j % 2
                h = hbuf[pl.ds(r0, RB), :]
                hn = _layernorm(h)
                gw = g[pl.ds(r0, RB + 16), :]
                gs = jnp.concatenate([
                    gw[7:7 + RB, 0:C], gw[9:9 + RB, C:2 * C], gw[6:6 + RB, 2 * C:3 * C], gw[10:10 + RB, 3 * C:]],
                    axis=1).astype(BF16)
                x1 = hn + jnp.dot(gs, w2[...], preferred_element_type=F32)
                y = _layernorm(x1).astype(BF16)
                a = _gelu(jnp.dot(y, w3[...], preferred_element_type=F32)).astype(BF16)
                h2 = jnp.dot(a, w4[...], preferred_element_type=F32)
                res = (h + (x1 + h2)).astype(BF16)

                @pl.when(j >= 2)
                def _():
                    out_copy(j - 2, slot).wait()
                obuf[slot] = res
                out_copy(j, slot).start()
                return carry
            nb = S // RB
            with jax.named_scope("PH_b2"):
                lax.fori_loop(0, nb, b2, 0)
            out_copy(nb - 2, nb % 2).wait()
            out_copy(nb - 1, (nb - 1) % 2).wait()

        pl.run_scoped(
            phase_b,
            pltpu.VMEM((S + 16, D), F32),
            pltpu.VMEM((2, RB, D), BF16),
        )

    return kernel


@functools.partial(jax.jit, static_argnames=("A_seg_len",))
def pallas_sequential_preLN__memory_aug_recurrent_mem_tr__mixer_s_mlp__prompt_kernel(A_x, A_mem0, A_Wq, A_Wk, A_Wv, A_Wo, A_seg_len, B_x, B_w1, B_w2, B_w3, B_w4):
    del B_x
    B, S, D = A_x.shape
    assert B == 1
    H, E = A_Wq.shape[1], A_Wq.shape[2]
    M = A_mem0.shape[1]
    FF = B_w3.shape[1]
    kern = _make_kernel(S, D, H, E, M, int(A_seg_len), FF)
    any_spec = pl.BlockSpec(memory_space=pl.ANY)
    out = pl.pallas_call(
        kern,
        out_shape=jax.ShapeDtypeStruct((S, D), A_x.dtype),
        in_specs=[any_spec] * 10,
        out_specs=any_spec,
        scratch_shapes=[
            pltpu.VMEM((S, D), BF16),
            pltpu.VMEM((M, D), BF16),
            pltpu.VMEM((S, D), F32),
            pltpu.VMEM((D, D), BF16),
            pltpu.VMEM((D, D), BF16),
            pltpu.VMEM((D, FF), BF16),
            pltpu.VMEM((FF, D), BF16),
            pltpu.SemaphoreType.DMA((2,)),
            pltpu.SemaphoreType.DMA((4,)),
            pltpu.SemaphoreType.DMA((2,)),
        ],
        compiler_params=pltpu.CompilerParams(vmem_limit_bytes=120 * 1024 * 1024),
    )(
        A_x.reshape(S, D), A_mem0.reshape(M, D),
        A_Wq.reshape(D * H, E), A_Wk.reshape(D * H, E), A_Wv.reshape(D * H, E),
        A_Wo.reshape(H * E, D), B_w1, B_w2, B_w3, B_w4,
    )
    return out.reshape(B, S, D)
```

```python
import functools
import math

import jax
import jax.numpy as jnp
from jax import lax
from jax.experimental import pallas as pl
from jax.experimental.pallas import tpu as pltpu

F32 = jnp.float32
BF16 = jnp.bfloat16
I32 = jnp.int32

LN_EPS = 1e-5
NEG = -1000000000.0

GH = int('4')
SCHED = 'pipe'
FLAGS = {k: True for k in ''.split(',') if k}
GROUPS = [tuple(int(c) for c in g.split('-')) for g in '0-1,1-2,2-4,4-8,8-16,16-24'.split(',')]
OSPLIT = [int(c) for c in '0,16,20,24,28,32'.split(',')]
SCOPES = '0' == '1'


class _NoScope:
    def __enter__(self):
        return self

    def __exit__(self, *a):
        return False


def _scope(name):
    return jax.named_scope(name) if SCOPES else _NoScope()


def _layernorm(x):
    m = jnp.mean(x, axis=-1, keepdims=True)
    c = x - m
    v = jnp.mean(c * c, axis=-1, keepdims=True)
    return c * lax.rsqrt(v + LN_EPS)


def _gelu(x):
    c0 = math.sqrt(2.0 / math.pi)
    u = x * (c0 + (c0 * 0.044715) * (x * x))
    return (0.5 * x) * (1.0 + jnp.tanh(u))


def _make_kernel(S, D, H, E, M, SEG, FF):
    NSEG = S // SEG
    LEFT = 8
    MAIN = SEG - LEFT
    RM = M + MAIN
    NL = NSEG * LEFT
    L = M + SEG
    LP = 128
    HE = H * E
    KC = 128
    NKC = D // KC
    NST = 3 * NKC
    HG = 4
    RB = 256
    scale = float(E) ** -0.5

    def kernel(x_hbm, mem_hbm, wq_hbm, wk_hbm, wv_hbm, wo_hbm, w1_hbm, w2_hbm, w3_hbm, w4_hbm,
               out_hbm,
               xs, mems, hbuf, wqkv, wo, lqkv, lo, sem_in, sem_wo):

        xl_cp = pltpu.make_async_copy(x_hbm.at[:, pl.ds(MAIN, LEFT), :], xs.at[:, pl.ds(MAIN, LEFT), :], sem_in.at[0])
        xm_cp = pltpu.make_async_copy(x_hbm.at[:, pl.ds(0, MAIN), :], xs.at[:, pl.ds(0, MAIN), :], sem_in.at[1])
        m_cp = pltpu.make_async_copy(mem_hbm, mems, sem_in.at[2])
        wo_cps = [pltpu.make_async_copy(wo_hbm.at[:, pl.ds(j * 128, 128)], wo.at[j], sem_wo.at[j])
                  for j in range(D // 128)]

        def w_head(j):
            return pltpu.bitcast(wqkv[j], BF16)

        def wo_full():
            return jnp.concatenate([wo[j] for j in range(D // 128)], axis=1)

        def prologue(stage, xl_s, sem_st):
            w_hbms = (wq_hbm, wk_hbm, wv_hbm)

            def st_copy(i):
                m, c = divmod(i, NKC)
                return pltpu.make_async_copy(
                    w_hbms[m].at[pl.ds(c * KC * H, KC * H), :], stage.at[i], sem_st.at[i])

            sub = lax.broadcasted_iota(I32, (8, E), 0)

            def t8x8(R):
                for sh in (4, 2, 1):
                    msk = (sub & sh) == 0
                    N = list(R)
                    for a in range(8):
                        if not a & sh:
                            N[a] = jnp.where(msk, R[a], pltpu.roll(R[a + sh], sh, 0))
                            N[a + sh] = jnp.where(msk, pltpu.roll(R[a], 8 - sh, 0), R[a + sh])
                    R = N
                return R

            def relayout(i):
                m, c = divmod(i, NKC)
                for half in range(H // 16):
                    for g in range(KC // 16):
                        orow = c * (KC // 2) + g * 8
                        U = []
                        for q in range(2):
                            r0 = [(g * 16 + q * 8 + j) * H + half * 16 for j in range(8)]
                            U.append(t8x8([pltpu.bitcast(stage[i, r:r + 16, :], I32) for r in r0]))
                        for t in range(8):
                            v = jnp.concatenate([U[0][t], U[1][t]], axis=0)
                            h = half * 16 + 2 * t
                            wqkv[m * H + h, orow:orow + 8, :] = pltpu.bitcast(v.astype(jnp.int16), I32)
                            wqkv[m * H + h + 1, orow:orow + 8, :] = pltpu.bitcast(
                                lax.shift_right_logical(v, 16).astype(jnp.int16), I32)

            def left_mm(i):
                m, c = divmod(i, NKC)
                for hg in range(H // HG):
                    w = jnp.concatenate(
                        [pltpu.bitcast(wqkv[m * H + hg * HG + t, c * (KC // 2):(c + 1) * (KC // 2), :], BF16)
                         for t in range(HG)], axis=1)
                    xc = pltpu.bitcast(xl_s[c], BF16)
                    r = jnp.dot(xc, w, preferred_element_type=F32)
                    cols = slice(hg * HG * E, (hg + 1) * HG * E)
                    if c == 0:
                        lqkv[m, :, cols] = r
                    else:
                        lqkv[m, :, cols] = lqkv[m, :, cols] + r

            groups = [range(a, b) for a, b in GROUPS]
            NGR = len(groups)

            def start_group(k):
                if k < NGR:
                    for i in groups[k]:
                        st_copy(i).start()
                if k == NGR - 2:
                    xm_cp.start()
                    m_cp.start()
                if k == NGR:
                    for cp in wo_cps:
                        cp.start()

            xl_cp.start()
            start_group(0)
            start_group(1)
            for k in range(NGR):
                with _scope("PH_left%d" % k):
                    if k == 0:
                        xl_cp.wait()
                    for i in groups[k]:
                        st_copy(i).wait()
                    start_group(k + 2)
                    if k == 0:
                        xl = _layernorm(xs[:, MAIN:, :].astype(F32).reshape(NL, D)).astype(BF16)
                        for c in range(NKC):
                            xl_s[c] = pltpu.bitcast(xl[:, c * KC:(c + 1) * KC], I32)
                    for i in groups[k]:
                        relayout(i)
                        left_mm(i)

        pl.run_scoped(
            prologue,
            pltpu.VMEM((NST, KC * H, E), BF16),
            pltpu.VMEM((NKC, NL // 2, KC), I32),
            pltpu.SemaphoreType.DMA((NST,)),
        )

        def rest(w1, w2, w3, w4, qkv_s, s_s, p_s, o_s, xn_s, sem_b, sem_out):
            b_cps = [pltpu.make_async_copy(a, b, sem_b.at[j])
                     for j, (a, b) in enumerate(((w1_hbm, w1), (w2_hbm, w2), (w3_hbm, w3), (w4_hbm, w4)))]
            with _scope("PH_wait"):
                xm_cp.wait()
                m_cp.wait()
                for cp in wo_cps:
                    cp.wait()
                for cp in b_cps:
                    cp.start()

            row = lax.broadcasted_iota(I32, (L, LP), 0)
            col = lax.broadcasted_iota(I32, (L, LP), 1)
            valid = (col < L) & ((row < M) | (row >= col))
            fill = jnp.where(col < L, NEG / scale, -jnp.inf).astype(F32)
            c_exp = scale * math.log2(math.e)

            def step(s, mem):
                r0 = pl.multiple_of(s * SEG, SEG)
                l0 = pl.multiple_of(s * LEFT, LEFT)
                lhs = jnp.concatenate([mem, xn_s[...]], axis=0).astype(BF16)

                def proj(h):
                    w = jnp.concatenate([w_head(h), w_head(H + h), w_head(2 * H + h)], axis=1)
                    qkv = jnp.dot(lhs, w, preferred_element_type=F32).astype(BF16)
                    for m in range(3):
                        qkv_s[m * H + h] = pltpu.bitcast(qkv[:, m * E:(m + 1) * E], I32)

                def full(m, h, rows):
                    main = pltpu.bitcast(qkv_s[m * H + h], BF16)
                    left = jnp.concatenate(
                        [lqkv[m, pl.ds(l0, LEFT), h * E:(h + 1) * E], jnp.zeros((8, E), F32)], axis=0).astype(BF16)
                    parts = [main, left]
                    if rows > RM + 16:
                        parts.append(jnp.zeros((rows - RM - 16, E), BF16))
                    return jnp.concatenate(parts, axis=0)

                def scores(h):
                    q = full(0, h, RM + 16)
                    k = full(1, h, LP)
                    sc = lax.dot_general(q, k, (((1,), (1,)), ((), ())), preferred_element_type=F32)
                    s_s[h] = sc[:L]

                def softmax(h):
                    sc = jnp.where(valid, s_s[h], fill)
                    mx = jnp.max(sc, axis=-1, keepdims=True)
                    e = jnp.exp2((sc - mx) * c_exp)
                    sm = jnp.sum(e, axis=-1, keepdims=True)
                    p = e * pl.reciprocal(sm, approx=True)
                    p = jnp.concatenate([p, jnp.zeros((8, LP), F32)], axis=0).astype(BF16)
                    p_s[h] = pltpu.bitcast(p, I32)

                def pv(h):
                    p = pltpu.bitcast(p_s[h], BF16)
                    v = full(2, h, LP)
                    o = jnp.dot(p, v, preferred_element_type=F32)
                    lo[pl.ds(l0, LEFT), h * E:(h + 1) * E] = o[RM:L, :]
                    o_s[:, h * E:(h + 1) * E] = pltpu.bitcast(o[:RM].astype(BF16), I32)

                acc = []

                def oproj(h0, h1):
                    o_p = pltpu.bitcast(o_s[:, h0 * E:h1 * E], BF16)
                    w = jnp.concatenate([wo[j, h0 * E:h1 * E, :] for j in range(D // 128)], axis=1)
                    r = jnp.dot(o_p, w, preferred_element_type=F32)
                    acc.append(r)

                NG = H // GH

                def grp(f, g):
                    if 0 <= g < NG:
                        for h in range(g * GH, (g + 1) * GH):
                            f(h)
                pieces = list(zip(OSPLIT[:-1], OSPLIT[1:]))
                for t in range(NG + 3):
                    grp(proj, t)
                    if t >= NG and pieces and pieces[0][1] <= (t - 3) * GH:
                        oproj(*pieces.pop(0))
                    grp(scores, t - 1)
                    grp(softmax, t - 2)
                    grp(pv, t - 3)
                while pieces:
                    oproj(*pieces.pop(0))
                out = acc[0]
                for r in acc[1:]:
                    out = out + r
                xr = xs[s, 0:MAIN, :].astype(F32)
                hbuf[pl.ds(r0, MAIN), :] = xr + out[M:, :]
                xn_s[...] = _layernorm(xs[jnp.minimum(s + 1, NSEG - 1), 0:MAIN, :].astype(F32))
                return out[:M, :]

            xn_s[...] = _layernorm(xs[0, 0:MAIN, :].astype(F32))
            with _scope("PH_main"):
                lax.fori_loop(0, NSEG, step, mems[...].astype(F32))

            with _scope("PH_oleft"):
                ol = jnp.dot(lo[...].astype(BF16), wo_full(), preferred_element_type=F32)
                for s in range(NSEG):
                    r = s * SEG + MAIN
                    hbuf[r:r + LEFT, :] = xs[s, MAIN:, :].astype(F32) + ol[s * LEFT:(s + 1) * LEFT, :]
                for cp in b_cps:
                    cp.wait()

            def phase_b(g, obuf):
                C = D // 4
                zeros = jnp.zeros((8, D), F32)
                g[0:8, :] = zeros
                g[S + 8:S + 16, :] = zeros

                def b1(j, carry):
                    r0 = pl.multiple_of(j * RB, RB)
                    hn = _layernorm(hbuf[pl.ds(r0, RB), :])
                    a = jnp.dot(hn.astype(BF16), w1[...], preferred_element_type=F32)
                    g[pl.ds(r0 + 8, RB), :] = _gelu(a)
                    return carry
                with _scope("PH_b1"):
                    lax.fori_loop(0, S // RB, b1, 0)

                def out_copy(j, slot):
                    return pltpu.make_async_copy(obuf.at[slot], out_hbm.at[pl.ds(j * RB, RB), :], sem_out.at[slot])

                def b2(j, carry):
                    r0 = pl.multiple_of(j * RB, RB)
                    slot = j % 2
                    h = hbuf[pl.ds(r0, RB), :]
                    hn = _layernorm(h)
                    gw = g[pl.ds(r0, RB + 16), :]
                    gs = jnp.concatenate([
                        gw[7:7 + RB, 0:C], gw[9:9 + RB, C:2 * C], gw[6:6 + RB, 2 * C:3 * C], gw[10:10 + RB, 3 * C:]],
                        axis=1).astype(BF16)
                    x1 = hn + jnp.dot(gs, w2[...], preferred_element_type=F32)
                    y = _layernorm(x1).astype(BF16)
                    a = _gelu(jnp.dot(y, w3[...], preferred_element_type=F32)).astype(BF16)
                    h2 = jnp.dot(a, w4[...], preferred_element_type=F32)
                    res = (h + (x1 + h2)).astype(BF16)

                    @pl.when(j >= 2)
                    def _():
                        out_copy(j - 2, slot).wait()
                    obuf[slot] = res
                    out_copy(j, slot).start()
                    return carry
                nb = S // RB
                with _scope("PH_b2"):
                    lax.fori_loop(0, nb, b2, 0)
                out_copy(nb - 2, nb % 2).wait()
                out_copy(nb - 1, (nb - 1) % 2).wait()

            pl.run_scoped(
                phase_b,
                pltpu.VMEM((S + 16, D), F32),
                pltpu.VMEM((2, RB, D), BF16),
            )

        pl.run_scoped(
            rest,
            pltpu.VMEM((D, D), BF16),
            pltpu.VMEM((D, D), BF16),
            pltpu.VMEM((D, FF), BF16),
            pltpu.VMEM((FF, D), BF16),
            pltpu.VMEM((3 * H, RM // 2, E), I32),
            pltpu.VMEM((H, L, LP), F32),
            pltpu.VMEM((H, 24, LP), I32),
            pltpu.VMEM((RM // 2, HE), I32),
            pltpu.VMEM((MAIN, D), F32),
            pltpu.SemaphoreType.DMA((4,)),
            pltpu.SemaphoreType.DMA((2,)),
        )

    scratch = [
        pltpu.VMEM((NSEG, SEG, D), BF16),
        pltpu.VMEM((M, D), BF16),
        pltpu.VMEM((S, D), F32),
        pltpu.VMEM((3 * H, D // 2, E), I32),
        pltpu.VMEM((D // 128, HE, 128), BF16),
        pltpu.VMEM((3, NL, HE), F32),
        pltpu.VMEM((NL, HE), F32),
        pltpu.SemaphoreType.DMA((3,)),
        pltpu.SemaphoreType.DMA((D // 128,)),
    ]
    return kernel, scratch


@functools.partial(jax.jit, static_argnames=("A_seg_len",))
def pallas_sequential_preLN__memory_aug_recurrent_mem_tr__mixer_s_mlp__prompt_kernel(A_x, A_mem0, A_Wq, A_Wk, A_Wv, A_Wo, A_seg_len, B_x, B_w1, B_w2, B_w3, B_w4):
    del B_x
    B, S, D = A_x.shape
    assert B == 1
    H, E = A_Wq.shape[1], A_Wq.shape[2]
    M = A_mem0.shape[1]
    FF = B_w3.shape[1]
    seg = int(A_seg_len)
    kern, scratch = _make_kernel(S, D, H, E, M, seg, FF)
    any_spec = pl.BlockSpec(memory_space=pl.ANY)
    out = pl.pallas_call(
        kern,
        out_shape=jax.ShapeDtypeStruct((S, D), A_x.dtype),
        in_specs=[any_spec] * 10,
        out_specs=any_spec,
        scratch_shapes=scratch,
        compiler_params=pltpu.CompilerParams(vmem_limit_bytes=124 * 1024 * 1024, flags=FLAGS or None),
    )(
        A_x.reshape(S // seg, seg, D), A_mem0.reshape(M, D),
        A_Wq.reshape(D * H, E), A_Wk.reshape(D * H, E), A_Wv.reshape(D * H, E),
        A_Wo.reshape(H * E, D), B_w1, B_w2, B_w3, B_w4,
    )
    return out.reshape(B, S, D)
```

```python
import functools
import math

import jax
import jax.numpy as jnp
from jax import lax
from jax.experimental import pallas as pl
from jax.experimental.pallas import tpu as pltpu

F32 = jnp.float32
BF16 = jnp.bfloat16
I32 = jnp.int32

LN_EPS = 1e-5
NEG = -1000000000.0

GH = int('4')
SCHED = 'pipe'
FLAGS = {k: True for k in ''.split(',') if k}
GROUPS = [tuple(int(c) for c in g.split('-')) for g in '0-1,1-2,2-4,4-8,8-16,16-24'.split(',')]
OSPLIT = [int(c) for c in '0,16,20,24,28,32'.split(',')]
BORD = int('1')
SHIFT = 'store'
STARTS = [[c for c in g.split('+') if c] for g in 'xl+0,1+2,3,4+xm,5,wo,'.split(',')]
UNROLL = int('2')
NSPLIT = int('0')
KSPLIT = int('768')
BU1 = int('1')
BU2 = int('0')
SCOPES = '0' == '1'


class _NoScope:
    def __enter__(self):
        return self

    def __exit__(self, *a):
        return False


def _scope(name):
    return jax.named_scope(name) if SCOPES else _NoScope()


def _layernorm(x):
    m = jnp.mean(x, axis=-1, keepdims=True)
    c = x - m
    v = jnp.mean(c * c, axis=-1, keepdims=True)
    return c * lax.rsqrt(v + LN_EPS)


def _gelu(x):
    c0 = math.sqrt(2.0 / math.pi)
    u = x * (c0 + (c0 * 0.044715) * (x * x))
    return (0.5 * x) * (1.0 + jnp.tanh(u))


def _make_kernel(S, D, H, E, M, SEG, FF):
    NSEG = S // SEG
    LEFT = 8
    MAIN = SEG - LEFT
    RM = M + MAIN
    NL = NSEG * LEFT
    L = M + SEG
    LP = 128
    HE = H * E
    KC = 128
    NKC = D // KC
    NST = 3 * NKC
    HG = 4
    RB = int('256')
    scale = float(E) ** -0.5

    def mult(v, n):
        return v if isinstance(v, int) else pl.multiple_of(v, n)

    def kernel(x_hbm, mem_hbm, wq_hbm, wk_hbm, wv_hbm, wo_hbm, w1_hbm, w2_hbm, w3_hbm, w4_hbm,
               out_hbm,
               xs, mems, hbuf, wqkv, wo, lqkv, lo, sem_in, sem_wo):

        xl_cp = pltpu.make_async_copy(x_hbm.at[:, pl.ds(MAIN, LEFT), :], xs.at[:, pl.ds(MAIN, LEFT), :], sem_in.at[0])
        xm_cp = pltpu.make_async_copy(x_hbm.at[:, pl.ds(0, MAIN), :], xs.at[:, pl.ds(0, MAIN), :], sem_in.at[1])
        m_cp = pltpu.make_async_copy(mem_hbm, mems, sem_in.at[2])
        wo_cps = [pltpu.make_async_copy(wo_hbm.at[:, pl.ds(j * 128, 128)], wo.at[j], sem_wo.at[j])
                  for j in range(D // 128)]

        def w_head(j):
            return pltpu.bitcast(wqkv[j], BF16)

        def wo_full():
            return jnp.concatenate([wo[j] for j in range(D // 128)], axis=1)

        def prologue(stage, xl_s, sem_st):
            w_hbms = (wq_hbm, wk_hbm, wv_hbm)

            def st_copy(i):
                m, c = divmod(i, NKC)
                return pltpu.make_async_copy(
                    w_hbms[m].at[pl.ds(c * KC * H, KC * H), :], stage.at[i], sem_st.at[i])

            sub = lax.broadcasted_iota(I32, (8, E), 0)

            def t8x8(R):
                for sh in (4, 2, 1):
                    msk = (sub & sh) == 0
                    N = list(R)
                    for a in range(8):
                        if not a & sh:
                            N[a] = jnp.where(msk, R[a], pltpu.roll(R[a + sh], sh, 0))
                            N[a + sh] = jnp.where(msk, pltpu.roll(R[a], 8 - sh, 0), R[a + sh])
                    R = N
                return R

            def relayout(i):
                m, c = divmod(i, NKC)
                for half in range(H // 16):
                    for g in range(KC // 16):
                        orow = c * (KC // 2) + g * 8
                        U = []
                        for q in range(2):
                            r0 = [(g * 16 + q * 8 + j) * H + half * 16 for j in range(8)]
                            U.append(t8x8([pltpu.bitcast(stage[i, r:r + 16, :], I32) for r in r0]))
                        for t in range(8):
                            v = jnp.concatenate([U[0][t], U[1][t]], axis=0)
                            h = half * 16 + 2 * t
                            wqkv[m * H + h, orow:orow + 8, :] = pltpu.bitcast(v.astype(jnp.int16), I32)
                            wqkv[m * H + h + 1, orow:orow + 8, :] = pltpu.bitcast(
                                lax.shift_right_logical(v, 16).astype(jnp.int16), I32)

            def left_mm(i):
                m, c = divmod(i, NKC)
                for hg in range(H // HG):
                    w = jnp.concatenate(
                        [pltpu.bitcast(wqkv[m * H + hg * HG + t, c * (KC // 2):(c + 1) * (KC // 2), :], BF16)
                         for t in range(HG)], axis=1)
                    xc = pltpu.bitcast(xl_s[c], BF16)
                    r = jnp.dot(xc, w, preferred_element_type=F32)
                    cols = slice(hg * HG * E, (hg + 1) * HG * E)
                    if c == 0:
                        lqkv[m, :, cols] = r
                    else:
                        lqkv[m, :, cols] = lqkv[m, :, cols] + r

            groups = [range(a, b) for a, b in GROUPS]
            NGR = len(groups)

            def start_items(items):
                for it in items:
                    if it == 'xm':
                        xm_cp.start()
                        m_cp.start()
                    elif it == 'wo':
                        for cp in wo_cps:
                            cp.start()
                    elif it == 'xl':
                        xl_cp.start()
                    else:
                        for i in groups[int(it)]:
                            st_copy(i).start()

            start_items(STARTS[0])
            for k in range(NGR):
                with _scope("PH_left%d" % k):
                    if k == 0:
                        xl_cp.wait()
                    for i in groups[k]:
                        st_copy(i).wait()
                    start_items(STARTS[k + 1])
                    if k == 0:
                        xl = _layernorm(xs[:, MAIN:, :].astype(F32).reshape(NL, D)).astype(BF16)
                        for c in range(NKC):
                            xl_s[c] = pltpu.bitcast(xl[:, c * KC:(c + 1) * KC], I32)
                    for i in groups[k]:
                        relayout(i)
                        left_mm(i)

        pl.run_scoped(
            prologue,
            pltpu.VMEM((NST, KC * H, E), BF16),
            pltpu.VMEM((NKC, NL // 2, KC), I32),
            pltpu.SemaphoreType.DMA((NST,)),
        )

        def rest(w1, w2, w3, w4, q_s, qkv_s, s_s, p_s, o_s, xn_s, sem_b, sem_out):
            b_cps = [pltpu.make_async_copy(a, b, sem_b.at[j])
                     for j, (a, b) in enumerate(((w1_hbm, w1), (w2_hbm, w2), (w3_hbm, w3), (w4_hbm, w4)))]
            with _scope("PH_wait"):
                xm_cp.wait()
                m_cp.wait()
                for cp in wo_cps:
                    cp.wait()
                for cp in b_cps:
                    cp.start()

            row = lax.broadcasted_iota(I32, (L, LP), 0)
            col = lax.broadcasted_iota(I32, (L, LP), 1)
            valid = (col < L) & ((row < M) | (row >= col))
            fill = jnp.where(col < L, NEG / scale, -jnp.inf).astype(F32)
            c_exp = scale * math.log2(math.e)

            def step(s, mem):
                l0 = mult(s * LEFT, LEFT)
                lhs = jnp.concatenate([mem, xn_s[...]], axis=0).astype(BF16)

                def proj(h):
                    w = jnp.concatenate([w_head(h), w_head(H + h), w_head(2 * H + h)], axis=1)
                    if h < NSPLIT:
                        qkv = (jnp.dot(lhs[:, :KSPLIT], w[:KSPLIT], preferred_element_type=F32)
                               + jnp.dot(lhs[:, KSPLIT:], w[KSPLIT:], preferred_element_type=F32))
                    else:
                        qkv = jnp.dot(lhs, w, preferred_element_type=F32)
                    q_s[h] = qkv[:, 0:E]
                    for m in (1, 2):
                        qkv_s[(m - 1) * H + h] = pltpu.bitcast(qkv[:, m * E:(m + 1) * E].astype(BF16), I32)

                def full(m, h, rows):
                    main = pltpu.bitcast(qkv_s[(m - 1) * H + h], BF16)
                    left = jnp.concatenate(
                        [lqkv[m, pl.ds(l0, LEFT), h * E:(h + 1) * E], jnp.zeros((8, E), F32)], axis=0).astype(BF16)
                    parts = [main, left]
                    if rows > RM + 16:
                        parts.append(jnp.zeros((rows - RM - 16, E), BF16))
                    return jnp.concatenate(parts, axis=0)

                def scores(h):
                    q = jnp.concatenate([q_s[h], lqkv[0, pl.ds(l0, LEFT), h * E:(h + 1) * E]], axis=0)
                    k = full(1, h, LP)
                    s_s[h] = lax.dot_general(q, k, (((1,), (1,)), ((), ())), preferred_element_type=F32)

                def softmax(h):
                    sc = jnp.where(valid, s_s[h], fill)
                    mx = jnp.max(sc, axis=-1, keepdims=True)
                    e = jnp.exp2((sc - mx) * c_exp)
                    sm = jnp.sum(e, axis=-1, keepdims=True)
                    p_s[h] = e * pl.reciprocal(sm, approx=True)

                def pv(h):
                    v = full(2, h, LP)
                    o = lax.dot_general(p_s[h], v, (((1,), (0,)), ((), ())), preferred_element_type=F32)
                    lo[pl.ds(l0, LEFT), h * E:(h + 1) * E] = o[RM:L, :]
                    o_s[:, h * E:(h + 1) * E] = pltpu.bitcast(o[:RM].astype(BF16), I32)

                acc = []

                def oproj(h0, h1):
                    o_p = pltpu.bitcast(o_s[:, h0 * E:h1 * E], BF16)
                    w = jnp.concatenate([wo[j, h0 * E:h1 * E, :] for j in range(D // 128)], axis=1)
                    r = jnp.dot(o_p, w, preferred_element_type=F32)
                    acc.append(r)

                NG = H // GH

                def grp(f, g):
                    if 0 <= g < NG:
                        for h in range(g * GH, (g + 1) * GH):
                            f(h)
                pieces = list(zip(OSPLIT[:-1], OSPLIT[1:]))
                for t in range(NG + 3):
                    grp(proj, t)
                    if t >= NG and pieces and pieces[0][1] <= (t - 3) * GH:
                        oproj(*pieces.pop(0))
                    grp(scores, t - 1)
                    grp(softmax, t - 2)
                    grp(pv, t - 3)
                while pieces:
                    oproj(*pieces.pop(0))
                out = acc[0]
                for r in acc[1:]:
                    out = out + r
                xr = xs[s, 0:MAIN, :].astype(F32)
                hbuf[s, 0:MAIN, :] = xr + out[M:, :]
                xn_s[...] = _layernorm(xs[jnp.minimum(s + 1, NSEG - 1), 0:MAIN, :].astype(F32))
                return out[:M, :]

            xn_s[...] = _layernorm(xs[0, 0:MAIN, :].astype(F32))
            def steps(t, mem, off=0):
                for u in range(UNROLL):
                    mem = step(t * UNROLL + u + off, mem)
                return mem

            with _scope("PH_main"):
                mem = mems[...].astype(F32)
                NPEEL = NSEG % UNROLL
                for u in range(NPEEL):
                    mem = step(u, mem)
                lax.fori_loop(0, NSEG // UNROLL, lambda t, m: steps(t, m, NPEEL), mem)

            with _scope("PH_oleft"):
                ol = jnp.dot(lo[...].astype(BF16), wo_full(), preferred_element_type=F32)
                hbuf[:, MAIN:, :] = xs[:, MAIN:, :].astype(F32) + ol.reshape(NSEG, LEFT, D)
                for cp in b_cps:
                    cp.wait()

            def phase_b(g, hn_s, y_s, gs_s):
                C = D // 4
                SB = RB // SEG
                nb = S // RB
                zeros = jnp.zeros((8, D), F32)
                g[0:8, :] = zeros
                g[8:16, :] = zeros
                g[S:S + 8, :] = zeros
                g[S + 8:S + 16, :] = zeros

                def h_block(j):
                    return hbuf[pl.ds(j * SB, SB)].reshape(RB, D)

                def ln_h(j, slot):
                    hn_s[j] = _layernorm(h_block(j)).astype(BF16)

                def mix1(j, slot):
                    a = jnp.dot(hn_s[j], w1[...], preferred_element_type=F32)
                    if SHIFT == 'store':
                        gw = g.at[pl.ds(mult(j * RB, RB), RB + 16), :]
                        a = _gelu(a)
                        for c, off in enumerate((9, 7, 10, 6)):
                            gw[off:off + RB, c * C:(c + 1) * C] = a[:, c * C:(c + 1) * C]
                    else:
                        g[pl.ds(mult(j * RB + 8, 8), RB), :] = _gelu(a)

                def b1(j, carry):
                    mix1(j, j % 2)
                    ln_h(j + 1, (j + 1) % 2)
                    return carry
                with _scope("PH_b1pre"):
                    ln_h(0, 0)
                with _scope("PH_b1"):
                    if BU1:
                        for j in range(nb - 1):
                            b1(j, 0)
                    else:
                        lax.fori_loop(0, nb - 1, b1, 0)
                with _scope("PH_b1post"):
                    mix1(nb - 1, (nb - 1) % 2)

                def out_copy(j):
                    return pltpu.make_async_copy(xs.at[pl.ds(j * SB, SB)], out_hbm.at[pl.ds(j * SB, SB)], sem_out.at[j])

                def shift(j):
                    r0 = mult(j * RB, RB)
                    if SHIFT == 'val':
                        gw = g[pl.ds(r0, RB + 16), :]
                    else:
                        gw = g.at[pl.ds(r0, RB + 16), :]
                    if SHIFT == 'store':
                        gs_s[...] = gw[8:8 + RB, :].astype(BF16)
                    else:
                        gs_s[...] = jnp.concatenate([
                            gw[7:7 + RB, 0:C], gw[9:9 + RB, C:2 * C], gw[6:6 + RB, 2 * C:3 * C], gw[10:10 + RB, 3 * C:]],
                            axis=1).astype(BF16)

                def mix2(j, slot, do_shift=True):
                    if do_shift:
                        shift(j)
                    h = h_block(j)
                    x1 = hn_s[j].astype(F32) + jnp.dot(gs_s[...], w2[...], preferred_element_type=F32)
                    y_s[slot] = _layernorm(x1).astype(BF16)
                    hbuf[pl.ds(j * SB, SB)] = (h + x1).reshape(SB, SEG, D)

                def mlp(j, slot):
                    a = _gelu(jnp.dot(y_s[slot], w3[...], preferred_element_type=F32)).astype(BF16)
                    h2 = jnp.dot(a, w4[...], preferred_element_type=F32)
                    xs[pl.ds(j * SB, SB)] = (h_block(j) + h2).astype(BF16).reshape(SB, SEG, D)
                    out_copy(j).start()

                def b2(j, carry):
                    if BORD == 0:
                        mix2(j + 1, (j + 1) % 2)
                        mlp(j, j % 2)
                    else:
                        slot = j % 2
                        if BORD == 2:
                            shift(j + 1)
                        a = _gelu(jnp.dot(y_s[slot], w3[...], preferred_element_type=F32)).astype(BF16)
                        mix2(j + 1, (j + 1) % 2, BORD != 2)
                        h2 = jnp.dot(a, w4[...], preferred_element_type=F32)
                        xs[pl.ds(j * SB, SB)] = (h_block(j) + h2).astype(BF16).reshape(SB, SEG, D)
                        out_copy(j).start()
                    return carry
                with _scope("PH_b2pre"):
                    mix2(0, 0)
                with _scope("PH_b2"):
                    if BU2:
                        for j in range(nb - 1):
                            b2(j, 0)
                    else:
                        lax.fori_loop(0, nb - 1, b2, 0)
                with _scope("PH_b2post"):
                    mlp(nb - 1, (nb - 1) % 2)
                for j in range(nb):
                    out_copy(j).wait()

            pl.run_scoped(
                phase_b,
                pltpu.VMEM((S + 16, D), F32),
                pltpu.VMEM((S // RB, RB, D), BF16),
                pltpu.VMEM((2, RB, D), BF16),
                pltpu.VMEM((RB, D), BF16),
            )

        pl.run_scoped(
            rest,
            pltpu.VMEM((D, D), BF16),
            pltpu.VMEM((D, D), BF16),
            pltpu.VMEM((D, FF), BF16),
            pltpu.VMEM((FF, D), BF16),
            pltpu.VMEM((H, RM, E), F32),
            pltpu.VMEM((2 * H, RM // 2, E), I32),
            pltpu.VMEM((H, L, LP), F32),
            pltpu.VMEM((H, L, LP), F32),
            pltpu.VMEM((RM // 2, HE), I32),
            pltpu.VMEM((MAIN, D), F32),
            pltpu.SemaphoreType.DMA((4,)),
            pltpu.SemaphoreType.DMA((S // RB,)),
        )

    scratch = [
        pltpu.VMEM((NSEG, SEG, D), BF16),
        pltpu.VMEM((M, D), BF16),
        pltpu.VMEM((NSEG, SEG, D), F32),
        pltpu.VMEM((3 * H, D // 2, E), I32),
        pltpu.VMEM((D // 128, HE, 128), BF16),
        pltpu.VMEM((3, NL, HE), F32),
        pltpu.VMEM((NL, HE), F32),
        pltpu.SemaphoreType.DMA((3,)),
        pltpu.SemaphoreType.DMA((D // 128,)),
    ]
    return kernel, scratch


@functools.partial(jax.jit, static_argnames=("A_seg_len",))
def pallas_sequential_preLN__memory_aug_recurrent_mem_tr__mixer_s_mlp__prompt_kernel(A_x, A_mem0, A_Wq, A_Wk, A_Wv, A_Wo, A_seg_len, B_x, B_w1, B_w2, B_w3, B_w4):
    del B_x
    B, S, D = A_x.shape
    assert B == 1
    H, E = A_Wq.shape[1], A_Wq.shape[2]
    M = A_mem0.shape[1]
    FF = B_w3.shape[1]
    seg = int(A_seg_len)
    kern, scratch = _make_kernel(S, D, H, E, M, seg, FF)
    any_spec = pl.BlockSpec(memory_space=pl.ANY)
    out = pl.pallas_call(
        kern,
        out_shape=jax.ShapeDtypeStruct((S // seg, seg, D), A_x.dtype),
        in_specs=[any_spec] * 10,
        out_specs=any_spec,
        scratch_shapes=scratch,
        compiler_params=pltpu.CompilerParams(vmem_limit_bytes=124 * 1024 * 1024, flags=FLAGS or None),
    )(
        A_x.reshape(S // seg, seg, D), A_mem0.reshape(M, D),
        A_Wq.reshape(D * H, E), A_Wk.reshape(D * H, E), A_Wv.reshape(D * H, E),
        A_Wo.reshape(H * E, D), B_w1, B_w2, B_w3, B_w4,
    )
    return out.reshape(B, S, D)
```

```python
import functools
import math

import jax
import jax.numpy as jnp
from jax import lax
from jax.experimental import pallas as pl
from jax.experimental.pallas import tpu as pltpu

F32 = jnp.float32
BF16 = jnp.bfloat16
I32 = jnp.int32

LN_EPS = 1e-5
MASKED = -1000000000.0
LANES = 128


def _layernorm(x):
    m = jnp.mean(x, axis=-1, keepdims=True)
    c = x - m
    v = jnp.mean(c * c, axis=-1, keepdims=True)
    return c * lax.rsqrt(v + LN_EPS)


def _gelu(x):
    c0 = math.sqrt(2.0 / math.pi)
    u = x * (c0 + (c0 * 0.044715) * (x * x))
    return (0.5 * x) * (1.0 + jnp.tanh(u))


def _dot(a, b):
    return jnp.dot(a, b, preferred_element_type=F32)


def _mult(v, n):
    return v if isinstance(v, int) else pl.multiple_of(v, n)


def _make_kernel(S, D, H, E, M, SEG, FF):
    NSEG = S // SEG
    LEFT = 8
    MAIN = SEG - LEFT
    RM = M + MAIN
    NL = NSEG * LEFT
    L = M + SEG
    HE = H * E
    KC = 128
    NKC = D // KC
    NST = 3 * NKC
    HG = 4
    GH = 4
    UNROLL = 3
    NSPLIT = 2
    KSPLIT = D // 2
    RB = 256
    SB = RB // SEG
    NB = S // RB
    LASTSPLIT = 2
    scale = float(E) ** -0.5
    assert (S, D, H, E, M, SEG) == (NSEG * SEG, D, H, LANES, 8, 32) and S % RB == 0
    assert D % (4 * LANES) == 0 and FF % LANES == 0 and H == 32 and D == 1024
    OSPLIT = (0, 12, 16, 20, 24, 28, 32)
    GROUPS = [range(a, b) for a, b in ((0, 1), (1, 2), (2, 4), (4, 8), (8, 14), (14, 24))]

    def kernel(x_hbm, mem_hbm, wq_hbm, wk_hbm, wv_hbm, wo_hbm, w1_hbm, w2_hbm, w3_hbm, w4_hbm,
               out_hbm,
               xs, mems, hbuf, wqkv, wo, lqkv, lo, sem_in, sem_wo):
        xl_cp = pltpu.make_async_copy(x_hbm.at[:, pl.ds(MAIN, LEFT), :], xs.at[:, pl.ds(MAIN, LEFT), :], sem_in.at[0])
        xm_cp = pltpu.make_async_copy(x_hbm.at[:, pl.ds(0, MAIN), :], xs.at[:, pl.ds(0, MAIN), :], sem_in.at[1])
        mem_cp = pltpu.make_async_copy(mem_hbm, mems, sem_in.at[2])
        wo_cps = [pltpu.make_async_copy(wo_hbm.at[:, pl.ds(j * LANES, LANES)], wo.at[j], sem_wo.at[j])
                  for j in range(D // LANES)]

        def w_head(j):
            return pltpu.bitcast(wqkv[j], BF16)

        def prologue(stage, xl_s, sem_st):
            w_hbms = (wq_hbm, wk_hbm, wv_hbm)

            def st_copy(i):
                m, c = divmod(i, NKC)
                return pltpu.make_async_copy(
                    w_hbms[m].at[pl.ds(c * KC * H, KC * H), :], stage.at[i], sem_st.at[i])

            sub = lax.broadcasted_iota(I32, (8, E), 0)

            def t8x8(R):
                for sh in (4, 2, 1):
                    msk = (sub & sh) == 0
                    N = list(R)
                    for a in range(8):
                        if not a & sh:
                            N[a] = jnp.where(msk, R[a], pltpu.roll(R[a + sh], sh, 0))
                            N[a + sh] = jnp.where(msk, pltpu.roll(R[a], 8 - sh, 0), R[a + sh])
                    R = N
                return R

            def relayout(i):
                m, c = divmod(i, NKC)
                for half in range(H // 16):
                    for g in range(KC // 16):
                        orow = c * (KC // 2) + g * 8
                        U = []
                        for q in range(2):
                            r0 = [(g * 16 + q * 8 + j) * H + half * 16 for j in range(8)]
                            U.append(t8x8([pltpu.bitcast(stage[i, r:r + 16, :], I32) for r in r0]))
                        for t in range(8):
                            v = jnp.concatenate([U[0][t], U[1][t]], axis=0)
                            h = m * H + half * 16 + 2 * t
                            wqkv[h, orow:orow + 8, :] = pltpu.bitcast(v.astype(jnp.int16), I32)
                            wqkv[h + 1, orow:orow + 8, :] = pltpu.bitcast(
                                lax.shift_right_logical(v, 16).astype(jnp.int16), I32)

            def left_mm(i):
                m, c = divmod(i, NKC)
                for hg in range(H // HG):
                    w = jnp.concatenate(
                        [pltpu.bitcast(wqkv[m * H + hg * HG + t, c * (KC // 2):(c + 1) * (KC // 2), :], BF16)
                         for t in range(HG)], axis=1)
                    r = _dot(pltpu.bitcast(xl_s[c], BF16), w)
                    cols = slice(hg * HG * E, (hg + 1) * HG * E)
                    if c == 0:
                        lqkv[m, :, cols] = r
                    else:
                        lqkv[m, :, cols] = lqkv[m, :, cols] + r

            def start_group(k):
                for i in GROUPS[k]:
                    st_copy(i).start()

            xl_cp.start()
            start_group(0)
            for k in range(len(GROUPS)):
                if k == 0:
                    xl_cp.wait()
                    nsb = 16 // LEFT
                    for b in range(NSEG // nsb):
                        xl = _layernorm(xs[b * nsb:(b + 1) * nsb, MAIN:, :].astype(F32).reshape(16, D)).astype(BF16)
                        for c in range(NKC):
                            xl_s[c, b * 8:(b + 1) * 8, :] = pltpu.bitcast(xl[:, c * KC:(c + 1) * KC], I32)
                for i in GROUPS[k]:
                    st_copy(i).wait()
                if k == 0:
                    start_group(1)
                if k + 2 < len(GROUPS):
                    start_group(k + 2)
                if k + 2 == len(GROUPS) - 2:
                    xm_cp.start()
                    mem_cp.start()
                if k + 2 == len(GROUPS):
                    for cp in wo_cps:
                        cp.start()
                for i in GROUPS[k]:
                    relayout(i)
                    left_mm(i)

        pl.run_scoped(
            prologue,
            pltpu.VMEM((NST, KC * H, E), BF16),
            pltpu.VMEM((NKC, NL // 2, KC), I32),
            pltpu.SemaphoreType.DMA((NST,)),
        )

        def rest(w1, w2, w3, w4, q_s, kv_s, s_s, p_s, o_s, xn_s, part_s, sem_b, sem_out):
            b_cps = [pltpu.make_async_copy(a, b, sem_b.at[j])
                     for j, (a, b) in enumerate(((w1_hbm, w1), (w2_hbm, w2), (w3_hbm, w3), (w4_hbm, w4)))]
            xm_cp.wait()
            mem_cp.wait()
            for cp in wo_cps:
                cp.wait()
            for cp in b_cps:
                cp.start()

            row = lax.broadcasted_iota(I32, (L, LANES), 0)
            col = lax.broadcasted_iota(I32, (L, LANES), 1)
            valid = (col < L) & ((row < M) | (row >= col))
            fill = jnp.where(col < L, MASKED / scale, -jnp.inf).astype(F32)
            c_exp = scale * math.log2(math.e)

            def step(s, mem):
                l0 = _mult(s * LEFT, LEFT)
                lhs = jnp.concatenate([mem, xn_s[...]], axis=0).astype(BF16)

                def w_qkv(h):
                    return jnp.concatenate([w_head(h), w_head(H + h), w_head(2 * H + h)], axis=1)

                def proj(h):
                    if h < NSPLIT:
                        if h == 0:
                            for h2 in range(NSPLIT):
                                part_s[h2] = _dot(lhs[:, :KSPLIT], w_qkv(h2)[:KSPLIT])
                        qkv = part_s[h] + _dot(lhs[:, KSPLIT:], w_qkv(h)[KSPLIT:])
                    else:
                        qkv = _dot(lhs, w_qkv(h))
                    q_s[h] = qkv[:, 0:E]
                    for m in (1, 2):
                        kv_s[(m - 1) * H + h] = pltpu.bitcast(qkv[:, m * E:(m + 1) * E].astype(BF16), I32)

                def keys_or_values(m, h):
                    main = pltpu.bitcast(kv_s[(m - 1) * H + h], BF16)
                    left = jnp.concatenate(
                        [lqkv[m, pl.ds(l0, LEFT), h * E:(h + 1) * E], jnp.zeros((16 - LEFT, E), F32)],
                        axis=0).astype(BF16)
                    return jnp.concatenate([main, left, jnp.zeros((LANES - RM - 16, E), BF16)], axis=0)

                def scores(h):
                    q = jnp.concatenate([q_s[h], lqkv[0, pl.ds(l0, LEFT), h * E:(h + 1) * E]], axis=0)
                    s_s[h] = lax.dot_general(q, keys_or_values(1, h), (((1,), (1,)), ((), ())),
                                             preferred_element_type=F32)

                def softmax(h):
                    sc = jnp.where(valid, s_s[h], fill)
                    mx = jnp.max(sc, axis=-1, keepdims=True)
                    e = jnp.exp2((sc - mx) * c_exp)
                    sm = jnp.sum(e, axis=-1, keepdims=True)
                    p_s[h] = e * pl.reciprocal(sm, approx=True)

                def pv(h):
                    o = lax.dot_general(p_s[h], keys_or_values(2, h), (((1,), (0,)), ((), ())),
                                        preferred_element_type=F32)
                    lo[pl.ds(l0, LEFT), h * E:(h + 1) * E] = o[RM:L, :]
                    o_s[:, h * E:(h + 1) * E] = pltpu.bitcast(o[:RM].astype(BF16), I32)

                acc = []

                def oproj(h0, h1):
                    w = jnp.concatenate([wo[j, h0 * E:h1 * E, :] for j in range(D // LANES)], axis=1)
                    acc.append(_dot(pltpu.bitcast(o_s[:, h0 * E:h1 * E], BF16), w))

                NG = H // GH

                def grp(f, g):
                    if 0 <= g < NG:
                        for h in range(g * GH, (g + 1) * GH):
                            f(h)

                pieces = list(zip(OSPLIT[:-1], OSPLIT[1:]))
                for t in range(NG + 3):
                    grp(proj, t)
                    if t >= NG and pieces and pieces[0][1] <= (t - 3) * GH:
                        oproj(*pieces.pop(0))
                    grp(scores, t - 1)
                    grp(softmax, t - 2)
                    grp(pv, t - 3)
                while pieces:
                    oproj(*pieces.pop(0))
                out = acc[0]
                for r in acc[1:]:
                    out = out + r
                hbuf[s, 0:MAIN, :] = xs[s, 0:MAIN, :].astype(F32) + out[M:, :]
                xn_s[...] = _layernorm(xs[jnp.minimum(s + 1, NSEG - 1), 0:MAIN, :].astype(F32))
                return out[:M, :]

            xn_s[...] = _layernorm(xs[0, 0:MAIN, :].astype(F32))
            mem = mems[...].astype(F32)
            NPEEL = NSEG % UNROLL
            for u in range(NPEEL):
                mem = step(u, mem)

            def steps(t, mem):
                for u in range(UNROLL):
                    mem = step(t * UNROLL + u + NPEEL, mem)
                return mem

            lax.fori_loop(0, NSEG // UNROLL, steps, mem)

            wo_all = jnp.concatenate([wo[j] for j in range(D // LANES)], axis=1)
            ol = _dot(lo[...].astype(BF16), wo_all)
            hbuf[:, MAIN:, :] = xs[:, MAIN:, :].astype(F32) + ol.reshape(NSEG, LEFT, D)
            for cp in b_cps:
                cp.wait()

            def phase_b(g, hn_s, y_s, gs_s):
                C = D // 4
                zeros = jnp.zeros((8, D), F32)
                g[0:8, :] = zeros
                g[8:16, :] = zeros
                g[S:S + 8, :] = zeros
                g[S + 8:S + 16, :] = zeros

                def h_block(j):
                    return hbuf[pl.ds(j * SB, SB)].reshape(RB, D)

                def ln_h(j):
                    hn_s[j] = _layernorm(h_block(j)).astype(BF16)

                def mix1(j):
                    a = _gelu(_dot(hn_s[j], w1[...]))
                    for c, off in enumerate((9, 7, 10, 6)):
                        g[j * RB + off:j * RB + off + RB, c * C:(c + 1) * C] = a[:, c * C:(c + 1) * C]

                ln_h(0)
                for j in range(NB):
                    mix1(j)
                    if j + 1 < NB:
                        ln_h(j + 1)

                def mix2(j, slot):
                    gs_s[...] = g[pl.ds(_mult(j * RB + 8, 8), RB), :].astype(BF16)
                    x1 = hn_s[j].astype(F32) + _dot(gs_s[...], w2[...])
                    y_s[slot] = _layernorm(x1).astype(BF16)
                    hbuf[pl.ds(j * SB, SB)] = (h_block(j) + x1).reshape(SB, SEG, D)

                def out_copy(j0, n, k):
                    return pltpu.make_async_copy(xs.at[pl.ds(j0, n)], out_hbm.at[pl.ds(j0, n)], sem_out.at[k])

                def block(j, carry):
                    a = _gelu(_dot(y_s[j % 2], w3[...])).astype(BF16)
                    mix2(j + 1, (j + 1) % 2)
                    h2 = _dot(a, w4[...])
                    xs[pl.ds(j * SB, SB)] = (h_block(j) + h2).astype(BF16).reshape(SB, SEG, D)
                    out_copy(j * SB, SB, j).start()
                    return carry

                mix2(0, 0)
                lax.fori_loop(0, NB - 1, block, 0)
                j = NB - 1
                n = SB // LASTSPLIT
                a = _gelu(_dot(y_s[j % 2], w3[...])).astype(BF16)
                for p in range(LASTSPLIT):
                    h2 = _dot(a[p * n * SEG:(p + 1) * n * SEG], w4[...])
                    hb = hbuf[pl.ds(j * SB + p * n, n)].reshape(n * SEG, D)
                    xs[pl.ds(j * SB + p * n, n)] = (hb + h2).astype(BF16).reshape(n, SEG, D)
                    out_copy(j * SB + p * n, n, j + p).start()
                for j in range(NB - 1):
                    out_copy(j * SB, SB, j).wait()
                for p in range(LASTSPLIT):
                    out_copy((NB - 1) * SB + p * n, n, NB - 1 + p).wait()

            pl.run_scoped(
                phase_b,
                pltpu.VMEM((S + 16, D), F32),
                pltpu.VMEM((NB, RB, D), BF16),
                pltpu.VMEM((2, RB, D), BF16),
                pltpu.VMEM((RB, D), BF16),
            )

        pl.run_scoped(
            rest,
            pltpu.VMEM((D, D), BF16),
            pltpu.VMEM((D, D), BF16),
            pltpu.VMEM((D, FF), BF16),
            pltpu.VMEM((FF, D), BF16),
            pltpu.VMEM((H, RM, E), F32),
            pltpu.VMEM((2 * H, RM // 2, E), I32),
            pltpu.VMEM((H, L, LANES), F32),
            pltpu.VMEM((H, L, LANES), F32),
            pltpu.VMEM((RM // 2, HE), I32),
            pltpu.VMEM((MAIN, D), F32),
            pltpu.VMEM((NSPLIT, RM, 3 * E), F32),
            pltpu.SemaphoreType.DMA((4,)),
            pltpu.SemaphoreType.DMA((NB - 1 + LASTSPLIT,)),
        )

    scratch = [
        pltpu.VMEM((NSEG, SEG, D), BF16),
        pltpu.VMEM((M, D), BF16),
        pltpu.VMEM((NSEG, SEG, D), F32),
        pltpu.VMEM((3 * H, D // 2, E), I32),
        pltpu.VMEM((D // LANES, HE, LANES), BF16),
        pltpu.VMEM((3, NL, HE), F32),
        pltpu.VMEM((NL, HE), F32),
        pltpu.SemaphoreType.DMA((3,)),
        pltpu.SemaphoreType.DMA((D // LANES,)),
    ]
    return kernel, scratch


@functools.partial(jax.jit, static_argnames=("A_seg_len",))
def pallas_sequential_preLN__memory_aug_recurrent_mem_tr__mixer_s_mlp__prompt_kernel(
    A_x: jax.Array,
    A_mem0: jax.Array,
    A_Wq: jax.Array,
    A_Wk: jax.Array,
    A_Wv: jax.Array,
    A_Wo: jax.Array,
    A_seg_len: int,
    B_x: jax.Array,
    B_w1: jax.Array,
    B_w2: jax.Array,
    B_w3: jax.Array,
    B_w4: jax.Array,
):
    del B_x
    B, S, D = A_x.shape
    assert B == 1
    H, E = A_Wq.shape[1], A_Wq.shape[2]
    M = A_mem0.shape[1]
    FF = B_w3.shape[1]
    seg = int(A_seg_len)
    kernel, scratch = _make_kernel(S, D, H, E, M, seg, FF)
    hbm = pl.BlockSpec(memory_space=pl.ANY)
    out = pl.pallas_call(
        kernel,
        out_shape=jax.ShapeDtypeStruct((S // seg, seg, D), A_x.dtype),
        in_specs=[hbm] * 10,
        out_specs=hbm,
        scratch_shapes=scratch,
        compiler_params=pltpu.CompilerParams(vmem_limit_bytes=124 * 1024 * 1024),
    )(
        A_x.reshape(S // seg, seg, D), A_mem0.reshape(M, D),
        A_Wq.reshape(D * H, E), A_Wk.reshape(D * H, E), A_Wv.reshape(D * H, E),
        A_Wo.reshape(H * E, D), B_w1, B_w2, B_w3, B_w4,
    )
    return out.reshape(B, S, D)
```

```python
import functools
import math

import jax
import jax.numpy as jnp
from jax import lax
from jax.experimental import pallas as pl
from jax.experimental.pallas import tpu as pltpu

F32 = jnp.float32
BF16 = jnp.bfloat16
I32 = jnp.int32

LN_EPS = 1e-5
MASKED = -1000000000.0
LANES = 128


def _layernorm(x):
    m = jnp.mean(x, axis=-1, keepdims=True)
    c = x - m
    v = jnp.mean(c * c, axis=-1, keepdims=True)
    return c * lax.rsqrt(v + LN_EPS)


def _gelu(x):
    c0 = math.sqrt(2.0 / math.pi)
    u = x * (c0 + (c0 * 0.044715) * (x * x))
    return (0.5 * x) * (1.0 + jnp.tanh(u))


def _dot(a, b):
    return jnp.dot(a, b, preferred_element_type=F32)


def _mult(v, n):
    return v if isinstance(v, int) else pl.multiple_of(v, n)


def _make_kernel(S, D, H, E, M, SEG, FF):
    NSEG = S // SEG
    LEFT = 8
    MAIN = SEG - LEFT
    RM = M + MAIN
    NL = NSEG * LEFT
    L = M + SEG
    HE = H * E
    KC = 128
    NKC = D // KC
    NST = 3 * NKC
    HG = 4
    GH = 4
    UNROLL = 3
    NSPLIT = 2
    KSPLIT = D // 2
    RB = 256
    SB = RB // SEG
    NB = S // RB
    LASTSPLIT = 2
    scale = float(E) ** -0.5
    assert (S, D, H, E, M, SEG) == (NSEG * SEG, D, H, LANES, 8, 32) and S % RB == 0
    assert D % (4 * LANES) == 0 and FF % LANES == 0 and H == 32 and D == 1024
    OSPLIT = (0, 12, 16, 20, 24, 28, 32)
    GROUPS = [range(a, b) for a, b in ((0, 1), (1, 2), (2, 4), (4, 8), (8, 14), (14, 24))]

    def kernel(x_hbm, mem_hbm, wq_hbm, wk_hbm, wv_hbm, wo_hbm, w1_hbm, w2_hbm, w3_hbm, w4_hbm,
               out_hbm,
               xs, mems, hbuf, wqkv, wo, lqkv, lo, sem_in, sem_wo):
        xl_cp = pltpu.make_async_copy(x_hbm.at[:, pl.ds(MAIN, LEFT), :], xs.at[:, pl.ds(MAIN, LEFT), :], sem_in.at[0])
        xm_cp = pltpu.make_async_copy(x_hbm.at[:, pl.ds(0, MAIN), :], xs.at[:, pl.ds(0, MAIN), :], sem_in.at[1])
        mem_cp = pltpu.make_async_copy(mem_hbm, mems, sem_in.at[2])
        wo_cps = [pltpu.make_async_copy(wo_hbm.at[:, pl.ds(j * LANES, LANES)], wo.at[j], sem_wo.at[j])
                  for j in range(D // LANES)]

        def w_head(j):
            return pltpu.bitcast(wqkv[j], BF16)

        def prologue(stage, xl_s, sem_st):
            w_hbms = (wq_hbm, wk_hbm, wv_hbm)

            def st_copy(i):
                m, c = divmod(i, NKC)
                return pltpu.make_async_copy(
                    w_hbms[m].at[pl.ds(c * KC * H, KC * H), :], stage.at[i], sem_st.at[i])

            sub = lax.broadcasted_iota(I32, (8, E), 0)

            def t8x8(R):
                for sh in (4, 2, 1):
                    msk = (sub & sh) == 0
                    N = list(R)
                    for a in range(8):
                        if not a & sh:
                            N[a] = jnp.where(msk, R[a], pltpu.roll(R[a + sh], sh, 0))
                            N[a + sh] = jnp.where(msk, pltpu.roll(R[a], 8 - sh, 0), R[a + sh])
                    R = N
                return R

            def relayout(i):
                m, c = divmod(i, NKC)
                for half in range(H // 16):
                    for g in range(KC // 16):
                        orow = c * (KC // 2) + g * 8
                        U = []
                        for q in range(2):
                            r0 = [(g * 16 + q * 8 + j) * H + half * 16 for j in range(8)]
                            U.append(t8x8([pltpu.bitcast(stage[i, r:r + 16, :], I32) for r in r0]))
                        for t in range(8):
                            v = jnp.concatenate([U[0][t], U[1][t]], axis=0)
                            h = m * H + half * 16 + 2 * t
                            wqkv[h, orow:orow + 8, :] = pltpu.bitcast(v.astype(jnp.int16), I32)
                            wqkv[h + 1, orow:orow + 8, :] = pltpu.bitcast(
                                lax.shift_right_logical(v, 16).astype(jnp.int16), I32)

            def left_mm(i):
                m, c = divmod(i, NKC)
                for hg in range(H // HG):
                    w = jnp.concatenate(
                        [pltpu.bitcast(wqkv[m * H + hg * HG + t, c * (KC // 2):(c + 1) * (KC // 2), :], BF16)
                         for t in range(HG)], axis=1)
                    r = _dot(pltpu.bitcast(xl_s[c], BF16), w)
                    cols = slice(hg * HG * E, (hg + 1) * HG * E)
                    if c == 0:
                        lqkv[m, :, cols] = r
                    else:
                        lqkv[m, :, cols] = lqkv[m, :, cols] + r

            def start_group(k):
                for i in GROUPS[k]:
                    st_copy(i).start()

            xl_cp.start()
            start_group(0)
            for k in range(len(GROUPS)):
                if k == 0:
                    xl_cp.wait()
                    nsb = 16 // LEFT
                    for b in range(NSEG // nsb):
                        xl = _layernorm(xs[b * nsb:(b + 1) * nsb, MAIN:, :].astype(F32).reshape(16, D)).astype(BF16)
                        for c in range(NKC):
                            xl_s[c, b * 8:(b + 1) * 8, :] = pltpu.bitcast(xl[:, c * KC:(c + 1) * KC], I32)
                for i in GROUPS[k]:
                    st_copy(i).wait()
                if k == 0:
                    start_group(1)
                if k + 2 < len(GROUPS):
                    start_group(k + 2)
                if k + 2 == len(GROUPS) - 2:
                    xm_cp.start()
                    mem_cp.start()
                if k + 2 == len(GROUPS):
                    for cp in wo_cps:
                        cp.start()
                for i in GROUPS[k]:
                    relayout(i)
                    left_mm(i)

        pl.run_scoped(
            prologue,
            pltpu.VMEM((NST, KC * H, E), BF16),
            pltpu.VMEM((NKC, NL // 2, KC), I32),
            pltpu.SemaphoreType.DMA((NST,)),
        )

        def rest(w1, w2, w3, w4, q_s, kv_s, s_s, p_s, o_s, xn_s, part_s, sem_b, sem_out):
            b_cps = [pltpu.make_async_copy(a, b, sem_b.at[j])
                     for j, (a, b) in enumerate(((w1_hbm, w1), (w2_hbm, w2), (w3_hbm, w3), (w4_hbm, w4)))]
            xm_cp.wait()
            mem_cp.wait()
            for cp in wo_cps:
                cp.wait()
            for cp in b_cps:
                cp.start()

            row = lax.broadcasted_iota(I32, (L, LANES), 0)
            col = lax.broadcasted_iota(I32, (L, LANES), 1)
            valid = (col < L) & ((row < M) | (row >= col))
            fill = jnp.where(col < L, MASKED / scale, -jnp.inf).astype(F32)
            c_exp = scale * math.log2(math.e)

            def step(s, mem):
                l0 = _mult(s * LEFT, LEFT)
                lhs = jnp.concatenate([mem, xn_s[...]], axis=0).astype(BF16)

                def w_qkv(h):
                    return jnp.concatenate([w_head(h), w_head(H + h), w_head(2 * H + h)], axis=1)

                def proj(h):
                    if h < NSPLIT:
                        if h == 0:
                            for h2 in range(NSPLIT):
                                part_s[h2] = _dot(lhs[:, :KSPLIT], w_qkv(h2)[:KSPLIT])
                        qkv = part_s[h] + _dot(lhs[:, KSPLIT:], w_qkv(h)[KSPLIT:])
                    else:
                        qkv = _dot(lhs, w_qkv(h))
                    q_s[h] = qkv[:, 0:E]
                    for m in (1, 2):
                        kv_s[(m - 1) * H + h] = pltpu.bitcast(qkv[:, m * E:(m + 1) * E].astype(BF16), I32)

                def keys_or_values(m, h):
                    main = pltpu.bitcast(kv_s[(m - 1) * H + h], BF16)
                    left = jnp.concatenate(
                        [lqkv[m, pl.ds(l0, LEFT), h * E:(h + 1) * E], jnp.zeros((16 - LEFT, E), F32)],
                        axis=0).astype(BF16)
                    return jnp.concatenate([main, left, jnp.zeros((LANES - RM - 16, E), BF16)], axis=0)

                def scores(h):
                    q = jnp.concatenate([q_s[h], lqkv[0, pl.ds(l0, LEFT), h * E:(h + 1) * E]], axis=0)
                    s_s[h] = lax.dot_general(q, keys_or_values(1, h), (((1,), (1,)), ((), ())),
                                             preferred_element_type=F32)

                def softmax(h):
                    sc = jnp.where(valid, s_s[h], fill)
                    mx = jnp.max(sc, axis=-1, keepdims=True)
                    e = jnp.exp2((sc - mx) * c_exp)
                    sm = jnp.sum(e, axis=-1, keepdims=True)
                    p_s[h] = e * pl.reciprocal(sm, approx=True)

                def pv(h):
                    o = lax.dot_general(p_s[h], keys_or_values(2, h), (((1,), (0,)), ((), ())),
                                        preferred_element_type=F32)
                    lo[pl.ds(l0, LEFT), h * E:(h + 1) * E] = o[RM:L, :]
                    o_s[:, h * E:(h + 1) * E] = pltpu.bitcast(o[:RM].astype(BF16), I32)

                acc = []

                def oproj(h0, h1):
                    w = jnp.concatenate([wo[j, h0 * E:h1 * E, :] for j in range(D // LANES)], axis=1)
                    acc.append(_dot(pltpu.bitcast(o_s[:, h0 * E:h1 * E], BF16), w))

                NG = H // GH

                def grp(f, g):
                    if 0 <= g < NG:
                        for h in range(g * GH, (g + 1) * GH):
                            f(h)

                pieces = list(zip(OSPLIT[:-1], OSPLIT[1:]))
                for t in range(NG + 3):
                    grp(proj, t)
                    if t >= NG and pieces and pieces[0][1] <= (t - 3) * GH:
                        oproj(*pieces.pop(0))
                    grp(scores, t - 1)
                    grp(softmax, t - 2)
                    grp(pv, t - 3)
                while pieces:
                    oproj(*pieces.pop(0))
                out = acc[0]
                for r in acc[1:]:
                    out = out + r
                hbuf[s, 0:MAIN, :] = xs[s, 0:MAIN, :].astype(F32) + out[M:, :]
                xn_s[...] = _layernorm(xs[jnp.minimum(s + 1, NSEG - 1), 0:MAIN, :].astype(F32))
                return out[:M, :]

            xn_s[...] = _layernorm(xs[0, 0:MAIN, :].astype(F32))
            mem = mems[...].astype(F32)
            NPEEL = NSEG % UNROLL
            for u in range(NPEEL):
                mem = step(u, mem)

            def steps(t, mem):
                for u in range(UNROLL):
                    mem = step(t * UNROLL + u + NPEEL, mem)
                return mem

            lax.fori_loop(0, NSEG // UNROLL, steps, mem)

            wo_all = jnp.concatenate([wo[j] for j in range(D // LANES)], axis=1)
            ol = _dot(lo[...].astype(BF16), wo_all)
            hbuf[:, MAIN:, :] = xs[:, MAIN:, :].astype(F32) + ol.reshape(NSEG, LEFT, D)
            for cp in b_cps:
                cp.wait()

            def phase_b(g, hn_s, y_s, gs_s):
                C = D // 4
                zeros = jnp.zeros((8, D), F32)
                g[0:8, :] = zeros
                g[8:16, :] = zeros
                g[S:S + 8, :] = zeros
                g[S + 8:S + 16, :] = zeros

                def h_block(j):
                    return hbuf[pl.ds(j * SB, SB)].reshape(RB, D)

                RH = RB // 2

                def ln_h(j, p):
                    hh = hbuf[pl.ds(j * SB + p * (SB // 2), SB // 2)].reshape(RH, D)
                    hn_s[j, p * RH:(p + 1) * RH, :] = _layernorm(hh).astype(BF16)

                def mix1(j, p):
                    a = _gelu(_dot(hn_s[j, p * RH:(p + 1) * RH, :], w1[...]))
                    r = j * RB + p * RH
                    for c, off in enumerate((9, 7, 10, 6)):
                        g[r + off:r + off + RH, c * C:(c + 1) * C] = a[:, c * C:(c + 1) * C]

                parts = [(j, p) for j in range(NB) for p in range(2)]
                ln_h(*parts[0])
                for i, jp in enumerate(parts):
                    mix1(*jp)
                    if i + 1 < len(parts):
                        ln_h(*parts[i + 1])

                def mix2(j, slot):
                    gs_s[...] = g[pl.ds(_mult(j * RB + 8, 8), RB), :].astype(BF16)
                    x1 = hn_s[j].astype(F32) + _dot(gs_s[...], w2[...])
                    y_s[slot] = _layernorm(x1).astype(BF16)
                    hbuf[pl.ds(j * SB, SB)] = (h_block(j) + x1).reshape(SB, SEG, D)

                def out_copy(j0, n, k):
                    return pltpu.make_async_copy(xs.at[pl.ds(j0, n)], out_hbm.at[pl.ds(j0, n)], sem_out.at[k])

                def block(j, carry):
                    a = _gelu(_dot(y_s[j % 2], w3[...])).astype(BF16)
                    mix2(j + 1, (j + 1) % 2)
                    h2 = _dot(a, w4[...])
                    xs[pl.ds(j * SB, SB)] = (h_block(j) + h2).astype(BF16).reshape(SB, SEG, D)
                    out_copy(j * SB, SB, j).start()
                    return carry

                mix2(0, 0)
                lax.fori_loop(0, NB - 1, block, 0)
                j = NB - 1
                n = SB // LASTSPLIT
                a = _gelu(_dot(y_s[j % 2], w3[...])).astype(BF16)
                for p in range(LASTSPLIT):
                    h2 = _dot(a[p * n * SEG:(p + 1) * n * SEG], w4[...])
                    hb = hbuf[pl.ds(j * SB + p * n, n)].reshape(n * SEG, D)
                    xs[pl.ds(j * SB + p * n, n)] = (hb + h2).astype(BF16).reshape(n, SEG, D)
                    out_copy(j * SB + p * n, n, j + p).start()
                for j in range(NB - 1):
                    out_copy(j * SB, SB, j).wait()
                for p in range(LASTSPLIT):
                    out_copy((NB - 1) * SB + p * n, n, NB - 1 + p).wait()

            pl.run_scoped(
                phase_b,
                pltpu.VMEM((S + 16, D), F32),
                pltpu.VMEM((NB, RB, D), BF16),
                pltpu.VMEM((2, RB, D), BF16),
                pltpu.VMEM((RB, D), BF16),
            )

        pl.run_scoped(
            rest,
            pltpu.VMEM((D, D), BF16),
            pltpu.VMEM((D, D), BF16),
            pltpu.VMEM((D, FF), BF16),
            pltpu.VMEM((FF, D), BF16),
            pltpu.VMEM((H, RM, E), F32),
            pltpu.VMEM((2 * H, RM // 2, E), I32),
            pltpu.VMEM((H, L, LANES), F32),
            pltpu.VMEM((H, L, LANES), F32),
            pltpu.VMEM((RM // 2, HE), I32),
            pltpu.VMEM((MAIN, D), F32),
            pltpu.VMEM((NSPLIT, RM, 3 * E), F32),
            pltpu.SemaphoreType.DMA((4,)),
            pltpu.SemaphoreType.DMA((NB - 1 + LASTSPLIT,)),
        )

    scratch = [
        pltpu.VMEM((NSEG, SEG, D), BF16),
        pltpu.VMEM((M, D), BF16),
        pltpu.VMEM((NSEG, SEG, D), F32),
        pltpu.VMEM((3 * H, D // 2, E), I32),
        pltpu.VMEM((D // LANES, HE, LANES), BF16),
        pltpu.VMEM((3, NL, HE), F32),
        pltpu.VMEM((NL, HE), F32),
        pltpu.SemaphoreType.DMA((3,)),
        pltpu.SemaphoreType.DMA((D // LANES,)),
    ]
    return kernel, scratch


@functools.partial(jax.jit, static_argnames=("A_seg_len",))
def pallas_sequential_preLN__memory_aug_recurrent_mem_tr__mixer_s_mlp__prompt_kernel(
    A_x: jax.Array,
    A_mem0: jax.Array,
    A_Wq: jax.Array,
    A_Wk: jax.Array,
    A_Wv: jax.Array,
    A_Wo: jax.Array,
    A_seg_len: int,
    B_x: jax.Array,
    B_w1: jax.Array,
    B_w2: jax.Array,
    B_w3: jax.Array,
    B_w4: jax.Array,
):
    del B_x
    B, S, D = A_x.shape
    assert B == 1
    H, E = A_Wq.shape[1], A_Wq.shape[2]
    M = A_mem0.shape[1]
    FF = B_w3.shape[1]
    seg = int(A_seg_len)
    kernel, scratch = _make_kernel(S, D, H, E, M, seg, FF)
    hbm = pl.BlockSpec(memory_space=pl.ANY)
    out = pl.pallas_call(
        kernel,
        out_shape=jax.ShapeDtypeStruct((S // seg, seg, D), A_x.dtype),
        in_specs=[hbm] * 10,
        out_specs=hbm,
        scratch_shapes=scratch,
        compiler_params=pltpu.CompilerParams(vmem_limit_bytes=124 * 1024 * 1024),
    )(
        A_x.reshape(S // seg, seg, D), A_mem0.reshape(M, D),
        A_Wq.reshape(D * H, E), A_Wk.reshape(D * H, E), A_Wv.reshape(D * H, E),
        A_Wo.reshape(H * E, D), B_w1, B_w2, B_w3, B_w4,
    )
    return out.reshape(B, S, D)
```
